```python
import os as _os
_os.environ.setdefault("JAX_PLATFORMS", "cpu")
import jax
import jax.numpy as jnp

def _softmax(x, axis=-1):
    return jax.nn.softmax(x, axis=axis)
def _gelu(x):
    return jax.nn.gelu(x, approximate=True)
def _silu(x):
    return jax.nn.silu(x)
def _sigmoid(x):
    return jax.nn.sigmoid(x)
def _layernorm(x, axis=-1, eps=1e-5):
    m = jnp.mean(x, axis=axis, keepdims=True)
    v = jnp.var(x, axis=axis, keepdims=True)
    return (x - m) / jnp.sqrt(v + eps)
def _scatter_add(tgt, idx, src, axis=0):
    return tgt.at[idx].add(src)
def _segment_sum(src, seg, n):
    return jax.ops.segment_sum(src, seg, n)
class _Rng:
    def __init__(self, key):
        self._k = key
    def _next(self):
        self._k, sub = jax.random.split(self._k)
        return sub
    def normal(self, shape):
        return jax.random.normal(self._next(), shape, dtype=jnp.bfloat16)
    def randint(self, lo, hi, shape):
        return jax.random.randint(self._next(), shape, lo, hi, dtype=jnp.int32)
    def uniform(self, shape, lo=0.0, hi=1.0):
        return jax.random.uniform(self._next(), shape, jnp.bfloat16, lo, hi)
    def permutation(self, n):
        return jax.random.permutation(self._next(), n)


kernel_name = 'interleave_layers__linear_kernel_hedgehog__ssm_conv_s4__prompt'

def setup_inputs():
    _rng = _Rng(jax.random.key(int.from_bytes(__import__("os").urandom(4), "little")))
    _w = (lambda a: (lambda t: t.astype(jnp.bfloat16) if jnp.issubdtype(t.dtype, jnp.floating) else t)(jnp.asarray(a)))
    def _A_setup():
        B, S, D, H = 1, 2048, 512, 32
        Dh = D // H
        return {
            "x": _w((lambda *s: _rng.normal(s) * 0.05)(B, S, D)),
            "wqkv": _w((lambda *s: _rng.normal(s) * 0.4)(D, 3 * D)),
            "w_phi": _w((lambda *s: _rng.normal(s) * 0.4)(H, Dh, Dh) * (Dh ** -0.5)),
            "wo": _w((lambda *s: _rng.normal(s) * 0.05)(D, D)),
        }
    _A_in = _A_setup()

    def _B_setup():
        B, L, D, N = 1, 2048, 512, 128
        A_re = -jnp.exp((lambda *s: _rng.normal(s) * 0.2)(D, N))
        A_im = jnp.pi * (lambda *s: _rng.normal(s) * 0.2)(D, N)
        B_re = (lambda *s: _rng.normal(s) * 0.2)(D, N)
        B_im = (lambda *s: _rng.normal(s) * 0.2)(D, N)
        C_re = (lambda *s: _rng.normal(s) * 0.2)(D, N)
        C_im = (lambda *s: _rng.normal(s) * 0.2)(D, N)
        log_dt = (lambda *s: _rng.normal(s) * 0.2)(D) * 0.5 - 4.0
        Dskip = (lambda *s: _rng.normal(s) * 0.2)(D)
        return {
            "u": _w((lambda *s: _rng.normal(s) * 0.05)(B, L, D)),
            "A_re": _w(A_re),
            "A_im": _w(A_im),
            "B_re": _w(B_re),
            "B_im": _w(B_im),
            "C_re": _w(C_re),
            "C_im": _w(C_im),
            "log_dt": _w(log_dt),
            "Dskip": _w(Dskip),
        }
    _B_in = _B_setup()

    return {
        "A_x": _A_in["x"],
        "A_wqkv": _A_in["wqkv"],
        "A_w_phi": _A_in["w_phi"],
        "A_wo": _A_in["wo"],
        "B_u": _B_in["u"],
        "B_A_re": _B_in["A_re"],
        "B_A_im": _B_in["A_im"],
        "B_B_re": _B_in["B_re"],
        "B_B_im": _B_in["B_im"],
        "B_C_re": _B_in["C_re"],
        "B_C_im": _B_in["C_im"],
        "B_log_dt": _B_in["log_dt"],
        "B_Dskip": _B_in["Dskip"],
    }

def reference(A_x, A_wqkv, A_w_phi, A_wo, B_u, B_A_re, B_A_im, B_B_re, B_B_im, B_C_re, B_C_im, B_log_dt, B_Dskip):
    def _A_ref(x, wqkv, w_phi, wo):
        B, S, D = x.shape
        H = 32; Dh = D // H
        qkv = (lambda x, *d: x.transpose(*d))((x @ wqkv).reshape(B, S, 3, H, Dh), 2, 0, 3, 1, 4)
        q, k, v = qkv[0], qkv[1], qkv[2]
        pq = jnp.einsum("bhsd,hdf->bhsf", q, w_phi)
        pk = jnp.einsum("bhsd,hdf->bhsf", k, w_phi)
        phi_q = jnp.concatenate([_softmax(pq, axis=-1), _softmax(-pq, axis=-1)], axis=-1)
        phi_k = jnp.concatenate([_softmax(pk, axis=-1), _softmax(-pk, axis=-1)], axis=-1)
        kv = jnp.einsum("bhsf,bhsd->bhfd", phi_k, v)
        z  = jnp.einsum("bhsf->bhf", phi_k)
        num = jnp.einsum("bhqf,bhfd->bhqd", phi_q, kv)
        den = jnp.einsum("bhqf,bhf->bhq", phi_q, z)[..., None] + 1e-6
        o = num / den
        return (lambda x, *d: x.transpose(*d))(o, 0, 2, 1, 3).reshape(B, S, D) @ wo

    def _B_ref(u, A_re, A_im, B_re, B_im, C_re, C_im, log_dt, Dskip):
        Bsz, L, D = u.shape
        dt = jnp.exp(log_dt)[:, None]
        A = A_re + 1j * A_im
        Bc = B_re + 1j * B_im
        Cc = C_re + 1j * C_im
        logdA = dt * A
        dB = dt * Bc
        l = (lambda x, dt: x.astype(dt))(jnp.arange(L), A_re.dtype)
        P = jnp.exp(logdA[:, :, None] * l[None, None, :])
        K = jnp.einsum("dn,dnl,dn->dl", Cc, P, dB).real
        L2 = 2 * L
        Kp = jnp.pad(K, ((0, 0), (0, L)))
        up = (lambda x, *d: x.transpose(*d))(u, 0, 2, 1)
        up = jnp.pad(up, ((0, 0), (0, 0), (0, L)))
        Kf = (lambda x, axes=(-2,-1): jnp.fft.rfft2(x.astype(jnp.float32), axes=axes))(Kp[:, None, :], axes=(-2, -1))
        Uf = (lambda x, axes=(-2,-1): jnp.fft.rfft2(x.astype(jnp.float32), axes=axes))(up[:, :, None, :], axes=(-2, -1))
        Yf = Uf * Kf[None, :, :, :]
        y = (lambda x, s, axes=(-2,-1): jnp.fft.irfft2(x, s=s, axes=axes).astype(jnp.bfloat16))(Yf, (1, L2), axes=(-2, -1))[:, :, 0, :L]
        y = (lambda x, *d: x.transpose(*d))(y, 0, 2, 1) + u * Dskip[None, None, :]
        return y

    x = A_x
    x = x + _A_ref(_layernorm(x, axis=-1), A_wqkv, A_w_phi, A_wo)
    x = x + _B_ref(_layernorm(x, axis=-1), B_A_re, B_A_im, B_B_re, B_B_im, B_C_re, B_C_im, B_log_dt, B_Dskip)
    x = x + _A_ref(_layernorm(x, axis=-1), A_wqkv, A_w_phi, A_wo)
    x = x + _B_ref(_layernorm(x, axis=-1), B_A_re, B_A_im, B_B_re, B_B_im, B_C_re, B_C_im, B_log_dt, B_Dskip)
    return x
```

```python
import jax
import jax.numpy as jnp
from jax import lax
import jax.experimental.pallas as pl
import jax.experimental.pallas.tpu as pltpu

S, D, H, DH, N = 2048, 512, 32, 16, 128
Q = 128
NC = S // Q
DP = D + 1
G = 8
F32, BF16, U32 = jnp.float32, jnp.bfloat16, jnp.uint32
NT = (((1,), (1,)), ((), ()))


def _dot(a, b):
    return jnp.dot(a, b, preferred_element_type=F32)


def _dot_nt(a, b):
    return lax.dot_general(a, b, NT, preferred_element_type=F32)


def _pack(x):
    return pltpu.bitcast(x, U32)


def _unpack(x):
    return pltpu.bitcast(x, BF16)


def _cmul(ar, ai, br, bi):
    return ar * br - ai * bi, ar * bi + ai * br


def _ln_t(x):
    m = jnp.mean(x, axis=0, keepdims=True)
    xc = x - m
    v = jnp.mean(xc * xc, axis=0, keepdims=True)
    return xc * lax.rsqrt(v + 1e-5)


def _feature_map(p):
    p = p.reshape(8, 8, 128)
    mx = jnp.max(p, axis=0)
    mn = jnp.min(p, axis=0)
    mx = jnp.maximum(mx, pltpu.roll(mx, 4, 0))
    mn = jnp.minimum(mn, pltpu.roll(mn, 4, 0))
    ep = jnp.exp(p - mx[None])
    en = jnp.exp(mn[None] - p)
    sp = jnp.sum(ep, axis=0)
    sn = jnp.sum(en, axis=0)
    sp = sp + pltpu.roll(sp, 4, 0)
    sn = sn + pltpu.roll(sn, 4, 0)
    ep = (ep * (1.0 / sp)[None]).reshape(64, 128)
    en = (en * (1.0 / sn)[None]).reshape(64, 128)
    return jnp.concatenate([ep, en], axis=0).astype(BF16)


def kernel_body(x_hbm, wqkv_hbm, wphi_ref, wo_hbm, are_ref, aim_ref, bre_ref, bim_ref,
                cre_ref, cim_ref, ldt_ref, dsk_ref, out_hbm,
                xin, wq_in, wo_in, wq_t, wkv_t, wo_t, X, U, Yb, xn_s, ph_s, ring, kv_s,
                ytab, Ur, ttab, pw, sbuf, hbuf, obuf, sems):
    cp_x = pltpu.make_async_copy(x_hbm, xin, sems.at[0])
    cp_w = pltpu.make_async_copy(wqkv_hbm, wq_in, sems.at[1])
    cp_o = pltpu.make_async_copy(wo_hbm, wo_in, sems.at[2])
    cp_w.start()
    cp_x.start()
    cp_o.start()

    dt = jnp.exp(ldt_ref[...].astype(F32)).astype(BF16).astype(F32)
    lr = dt * are_ref[...].astype(F32)
    li = dt * aim_ref[...].astype(F32)
    mag = jnp.exp(lr)
    pr, pi = mag * jnp.cos(li), mag * jnp.sin(li)
    for k in range(8):
        pw[0, k] = pr
        pw[1, k] = pi
        pr, pi = pr * pr - pi * pi, 2.0 * pr * pi
    wr, wi = _cmul(cre_ref[...].astype(F32), cim_ref[...].astype(F32),
                   dt * bre_ref[...].astype(F32), dt * bim_ref[...].astype(F32))
    pw[0, 8] = wr
    pw[1, 8] = wi
    w1r, w1i = _cmul(wr, wi, pw[0, 0], pw[1, 0])
    pw[0, 9] = w1r
    pw[1, 9] = w1i
    lane0 = lax.broadcasted_iota(jnp.int32, (D, N), 1) == 0
    pw[0, 10] = jnp.where(lane0, dsk_ref[...].astype(F32), 0.0)
    Ur[0:D, :] = jnp.zeros((D, Q), F32)
    rev_idx = 127 - lax.broadcasted_iota(jnp.int32, (D, Q), 1)

    row8 = lax.broadcasted_iota(jnp.int32, (8, 128), 0)

    def gen_tables(d):
        def bc(part, k):
            return jnp.broadcast_to(pw[part, k, pl.ds(d, 1), :], (8, 128))
        one = jnp.ones((8, 128), F32)
        zero = jnp.zeros((8, 128), F32)
        b0 = (row8 & 1) != 0
        yr = jnp.where(b0, bc(0, 0), one)
        yi = jnp.where(b0, bc(1, 0), zero)
        for k in (1, 2):
            tr, ti = _cmul(yr, yi, bc(0, k), bc(1, k))
            bk = (row8 & (1 << k)) != 0
            yr = jnp.where(bk, tr, yr)
            yi = jnp.where(bk, ti, yi)
        rs, is_ = [yr], [yi]
        for k in (3, 4, 5, 6):
            mr, mi = bc(0, k), bc(1, k)
            for j in range(len(rs)):
                tr, ti = _cmul(rs[j], is_[j], mr, mi)
                rs.append(tr)
                is_.append(ti)
        yr = jnp.concatenate(rs, axis=0).astype(BF16)
        yi = jnp.concatenate(is_, axis=0).astype(BF16)
        ytab[d, :, 0:128] = yr
        ytab[d, :, 128:256] = yi

    cp_w.wait()
    r128 = lax.broadcasted_iota(jnp.int32, (128, 128), 0)
    c128 = lax.broadcasted_iota(jnp.int32, (128, 128), 1)
    r16 = lax.broadcasted_iota(jnp.int32, (128, 16), 0)
    c16 = lax.broadcasted_iota(jnp.int32, (128, 16), 1)
    sel = (((r16 % 64) // 4) == c16).astype(BF16)
    hmask = ((r128 // 64) * 4 + r128 % 4) == (c128 // 16)
    for j in range(4):
        e = _dot_nt(sel, wphi_ref[j * 128:(j + 1) * 128, :])
        e = jnp.where(hmask, e, 0.0).astype(BF16)
        wq_t[j * 64:(j + 1) * 64, :] = _pack(
            _dot_nt(e, wq_in[:, j * 128:(j + 1) * 128]).astype(BF16))
        wkv_t[j * 64:(j + 1) * 64, :] = _pack(
            _dot_nt(e, wq_in[:, D + j * 128:D + (j + 1) * 128]).astype(BF16))
    wkv_t[256:512, :] = _pack(wq_in[:, 2 * D:3 * D].astype(F32).T.astype(BF16))
    cp_o.wait()
    wo_t[...] = _pack(wo_in[...].astype(F32).T.astype(BF16))
    cp_x.wait()

    kvmask = (lax.broadcasted_iota(jnp.int32, (80, 128), 0) // 16
              == lax.broadcasted_iota(jnp.int32, (80, 128), 1) % 4)
    zrow = lax.broadcasted_iota(jnp.int32, (80, 128), 0) >= 64
    zmask = ((lax.broadcasted_iota(jnp.int32, (80, 128), 0) % 4)
             == lax.broadcasted_iota(jnp.int32, (80, 128), 1) % 4)

    def attn_layer(first):
        kv_s[...] = jnp.zeros(kv_s.shape, F32)

        def norm_in(c, live=True):
            if first:
                xt = xin[pl.ds(pl.multiple_of(c * Q, Q), Q), :].astype(F32).T
            else:
                xt = X[c] + jnp.where(live, Yb[pl.ds(c * DP, D), :], 0.0)
            X[c] = xt
            xn_s[c] = _ln_t(xt).astype(BF16)

        def pass1(c, carry):
            xn = xn_s[c]
            kvp = _dot(_unpack(wkv_t[...]), xn)
            qp = _dot(_unpack(wq_t[...]), xn)
            ones = jnp.ones((16, 128), BF16)
            for hg in range(8):
                ph = _feature_map(kvp[hg * 64:(hg + 1) * 64])
                v = jnp.concatenate([kvp[D + hg * 64:D + (hg + 1) * 64].astype(BF16), ones], axis=0)
                kv_s[hg] += _dot_nt(v, ph)
                if first:
                    gen_tables(c * 16 + hg)
            for hg in range(8):
                ph_s[c, hg * 128:(hg + 1) * 128, :] = _feature_map(qp[hg * 64:(hg + 1) * 64])
                if first:
                    gen_tables(c * 16 + 8 + hg)
            norm_in(jnp.minimum(c + 1, NC - 1), c + 1 < NC)
            return carry
        norm_in(0)
        lax.fori_loop(0, NC, pass1, 0)

        kvb = []
        for hg in range(8):
            t = kv_s[hg]
            t = jnp.where(zrow, jnp.where(zmask, t, 0.0), jnp.where(kvmask, t, 0.0))
            kvb.append(t.astype(BF16))

        def out_proj(c):
            os_ = []
            for hg in range(8):
                nd = _dot(kvb[hg], ph_s[c, hg * 128:(hg + 1) * 128, :])
                r = 1.0 / (nd[64:72] + 1e-6)
                for h4 in range(4):
                    os_.append(nd[h4 * 16:(h4 + 1) * 16] * r[h4:h4 + 1])
            o = jnp.concatenate(os_, axis=0).astype(BF16)
            X[c] = X[c] + _dot(_unpack(wo_t[...]), o)

        def norm_out(c):
            u = _ln_t(X[c])
            U[pl.ds(c * DP, D), :] = u
            Ur[pl.ds((c + 1) * DP, D), :] = jnp.take_along_axis(u, rev_idx, axis=1)

        def pass2(c, carry):
            norm_out(jnp.maximum(c - 1, 0))
            out_proj(c)
            if first:
                for j in range(16):
                    gen_tables(D // 2 + c * 16 + j)
            return carry
        lax.fori_loop(0, NC, pass2, 0, unroll=2)

        norm_out(NC - 1)

    trow = lax.broadcasted_iota(jnp.int32, (128, 128), 0)
    tcol = lax.broadcasted_iota(jnp.int32, (128, 128), 1)

    def ssm_layer(first):
        def stage_a(g):
            sl = g % 2
            for j in range(G):
                d = g * G + j
                ur = Ur[pl.ds(d, NC, stride=DP), :].astype(BF16)
                s = _dot(ur, ytab[d])
                sbuf[sl, 0, pl.ds(j, NC, stride=G + 1), :] = s[:, 0:128]
                sbuf[sl, 1, pl.ds(j, NC, stride=G + 1), :] = s[:, 128:256]
                if not first:
                    u = U[pl.ds(d, NC, stride=DP), :].astype(BF16)
                    ring[sl, j * NC:(j + 1) * NC, :] = _dot(u, ttab[d])

        def stage_b(g):
            sl = g % 2
            d0 = pl.multiple_of(g * G, G)
            lr_, li_ = pw[0, 7, pl.ds(d0, G), :], pw[1, 7, pl.ds(d0, G), :]
            w1r_, w1i_ = pw[0, 9, pl.ds(d0, G), :], pw[1, 9, pl.ds(d0, G), :]
            hr = sbuf[sl, 0, 0:G, :]
            hi = sbuf[sl, 1, 0:G, :]
            for c in range(NC):
                if c > 0:
                    tr, ti = _cmul(hr, hi, lr_, li_)
                    hr = tr + sbuf[sl, 0, c * (G + 1):c * (G + 1) + G, :]
                    hi = ti + sbuf[sl, 1, c * (G + 1):c * (G + 1) + G, :]
                gr, gi = _cmul(hr, hi, w1r_, w1i_)
                hbuf[sl, 0, pl.ds(c, G, stride=33), :] = gr
                hbuf[sl, 1, pl.ds(c, G, stride=33), :] = -gi
            if first:
                hbuf[sl, 0, pl.ds(16, G, stride=33), :] = pw[0, 8, pl.ds(d0, G), :]
                hbuf[sl, 1, pl.ds(16, G, stride=33), :] = -pw[1, 8, pl.ds(d0, G), :]

        def stage_c(g):
            sl = g % 2
            nr = 32 if first else 16
            for j in range(G):
                d = g * G + j
                hw = jnp.concatenate([hbuf[sl, 0, j * 33:j * 33 + nr, :],
                                      hbuf[sl, 1, j * 33:j * 33 + nr, :]], axis=1).astype(BF16)
                yk = _dot_nt(hw, ytab[d])
                if first:
                    krow = yk[16:17] + pw[0, 10, pl.ds(d, 1), :]
                    t = pltpu.roll(jnp.broadcast_to(krow, (128, 128)), 0, 1, stride=1, stride_axis=0)
                    ttab[d] = jnp.where(tcol >= trow, t, 0.0).astype(BF16)
                    ring[sl, j * NC:(j + 1) * NC, :] = yk[0:16]
                else:
                    Yb[pl.ds(d, NC, stride=DP), :] = yk + ring[sl, j * NC:(j + 1) * NC, :]

        def stage_d(g):
            sl = g % 2
            for j in range(G):
                d = g * G + j
                u = U[pl.ds(d, NC, stride=DP), :].astype(BF16)
                Yb[pl.ds(d, NC, stride=DP), :] = ring[sl, j * NC:(j + 1) * NC, :] + _dot(u, ttab[d])

        stages = [stage_a, stage_b, stage_c] + ([stage_d] if first else [])
        ns, ng = len(stages), D // G
        def run(t, valid):
            for k in reversed(range(ns)):
                if valid(k):
                    stages[k](t - k)
        for t in range(ns - 1):
            run(t, lambda k: k <= t)

        step = 1 if first else 2
        npair = (ng - (ns - 1)) // step

        def body(i, carry):
            for r in range(step):
                run(ns - 1 + step * i + r, lambda k: True)
            return carry
        lax.fori_loop(0, npair, body, 0)
        for t in range(ns - 1 + step * npair, ng):
            run(t, lambda k: True)
        for t in range(ng, ng + ns - 1):
            run(t, lambda k: t - k < ng)

    hbuf[...] = jnp.zeros(hbuf.shape, F32)

    attn_layer(True)
    ssm_layer(True)
    attn_layer(False)
    ssm_layer(False)

    def out_copy(c):
        rows = pl.ds(pl.multiple_of(c * Q, Q), Q)
        return pltpu.make_async_copy(obuf.at[rows], out_hbm.at[rows], sems.at[0])

    def fin(c, carry):
        xt = X[c] + Yb[pl.ds(c * DP, D), :]
        obuf[pl.ds(pl.multiple_of(c * Q, Q), Q), :] = xt.T.astype(BF16)
        out_copy(c).start()
        return carry
    lax.fori_loop(0, NC, fin, 0)

    def drain(c, carry):
        out_copy(c).wait()
        return carry
    lax.fori_loop(0, NC, drain, 0)


@jax.jit
def pallas_interleave_layers__linear_kernel_hedgehog__ssm_conv_s4__prompt_kernel(
    A_x, A_wqkv, A_w_phi, A_wo, B_u, B_A_re, B_A_im, B_B_re, B_B_im, B_C_re, B_C_im,
    B_log_dt, B_Dskip,
):
    del B_u
    anyspec = pl.BlockSpec(memory_space=pl.ANY)
    vm = pl.BlockSpec(memory_space=pltpu.VMEM)
    out = pl.pallas_call(
        kernel_body,
        out_shape=jax.ShapeDtypeStruct((S, D), BF16),
        in_specs=[anyspec, anyspec, vm, anyspec] + [vm] * 8,
        out_specs=anyspec,
        scratch_shapes=[
            pltpu.VMEM((S, D), BF16),
            pltpu.VMEM((D, 3 * D), BF16),
            pltpu.VMEM((D, D), BF16),
            pltpu.VMEM((D // 2, D), U32),
            pltpu.VMEM((D, D), U32),
            pltpu.VMEM((D // 2, D), U32),
            pltpu.VMEM((NC, D, Q), F32),
            pltpu.VMEM((NC * DP + 7, Q), F32),
            pltpu.VMEM((NC * DP + 7, Q), F32),
            pltpu.VMEM((NC, D, Q), BF16),
            pltpu.VMEM((NC, 2 * D, Q), BF16),
            pltpu.VMEM((2, G * NC, Q), F32),
            pltpu.VMEM((8, 80, 128), F32),
            pltpu.VMEM((D, Q, 256), BF16),
            pltpu.VMEM(((NC + 1) * DP + 7, Q), F32),
            pltpu.VMEM((D, Q, Q), BF16),
            pltpu.VMEM((2, 11, D, N), F32),
            pltpu.VMEM((2, 2, NC * (G + 1), 128), F32),
            pltpu.VMEM((2, 2, G * 33 + 7, 128), F32),
            pltpu.VMEM((S, D), BF16),
            pltpu.SemaphoreType.DMA((3,)),
        ],
        compiler_params=pltpu.CompilerParams(vmem_limit_bytes=120 * 2 ** 20),
    )(A_x.reshape(S, D), A_wqkv, A_w_phi.reshape(H * DH, DH), A_wo,
      B_A_re, B_A_im, B_B_re, B_B_im, B_C_re, B_C_im,
      B_log_dt.reshape(D, 1), B_Dskip.reshape(D, 1))
    return out.reshape(1, S, D)
```
